```python
import jax
import jax.numpy as jnp

def _softmax(x, axis=-1):
    return jax.nn.softmax(x, axis=axis)
def _gelu(x):
    return jax.nn.gelu(x, approximate=True)
def _silu(x):
    return jax.nn.silu(x)
def _sigmoid(x):
    return jax.nn.sigmoid(x)
def _layernorm(x, axis=-1, eps=1e-5):
    m = jnp.mean(x, axis=axis, keepdims=True)
    v = jnp.var(x, axis=axis, keepdims=True)
    return (x - m) / jnp.sqrt(v + eps)
def _scatter_add(tgt, idx, src, axis=0):
    return tgt.at[idx].add(src)
def _segment_sum(src, seg, n):
    return jax.ops.segment_sum(src, seg, n)
class _Rng:
    def __init__(self, key):
        self._k = key
    def _next(self):
        self._k, sub = jax.random.split(self._k)
        return sub
    def normal(self, shape):
        return jax.random.normal(self._next(), shape, dtype=jnp.bfloat16)
    def randint(self, lo, hi, shape):
        return jax.random.randint(self._next(), shape, lo, hi, dtype=jnp.int32)
    def uniform(self, shape, lo=0.0, hi=1.0):
        return jax.random.uniform(self._next(), shape, jnp.bfloat16, lo, hi)
    def permutation(self, n):
        return jax.random.permutation(self._next(), n)


kernel_name = 'interleave_layers__sliding_block_cached__moe_arch_mod__decode'

def setup_inputs():
    _rng = _Rng(jax.random.key(int.from_bytes(__import__("os").urandom(4), "little")))
    _w = (lambda a: (lambda t: t.astype(jnp.bfloat16) if jnp.issubdtype(t.dtype, jnp.floating) else t)(jnp.asarray(a)))
    def _A_setup():
        B, Sq, D = 4, 1, 640
        Hq, Hkv, Sk, Dh = 32, 32, 4096, 192
        assert Hq % Hkv == 0, (Hq, Hkv)
        return {
            "x": _w((lambda *s: _rng.normal(s) * 0.05)(B, Sq, D)),
            "k_cache": _w((lambda *s: _rng.normal(s) * 0.05)(B, Hkv, Sk, Dh)),
            "v_cache": _w((lambda *s: _rng.normal(s) * 0.05)(B, Hkv, Sk, Dh)),
            "wq": _w((lambda *s: _rng.normal(s) * 0.05)(D, Hq * Dh) * (D ** -0.5)),
            "wo": _w((lambda *s: _rng.normal(s) * 0.05)(Hq * Dh, D) * ((Hq * Dh) ** -0.5)),
        }
    _A_in = _A_setup()

    def _B_setup():
        B, S, D, F, C = 4, 1, 640, 1536, 1
        return {
            "x": _w((lambda *s: _rng.normal(s) * 0.05)(B, S, D)),
            "w_r": _w((lambda *s: _rng.normal(s) * 0.05)(D)),
            "w_gate": _w((lambda *s: _rng.normal(s) * 0.05)(D, F)),
            "w_up": _w((lambda *s: _rng.normal(s) * 0.05)(D, F)),
            "w_down": _w((lambda *s: _rng.normal(s) * 0.05)(F, D)),
        }
    _B_in = _B_setup()

    return {
        "A_x": _A_in["x"],
        "A_k_cache": _A_in["k_cache"],
        "A_v_cache": _A_in["v_cache"],
        "A_wq": _A_in["wq"],
        "A_wo": _A_in["wo"],
        "B_x": _B_in["x"],
        "B_w_r": _B_in["w_r"],
        "B_w_gate": _B_in["w_gate"],
        "B_w_up": _B_in["w_up"],
        "B_w_down": _B_in["w_down"],
    }

def reference(A_x, A_k_cache, A_v_cache, A_wq, A_wo, B_x, B_w_r, B_w_gate, B_w_up, B_w_down):
    def _A_ref(x, k_cache, v_cache, wq, wo):
        B, Sq, D = x.shape
        Hq, Dh = 32, 192
        Hkv, Sk = k_cache.shape[1], k_cache.shape[2]
        W = min(4096, max(256, Sk // 4))
        rep = Hq // Hkv
        q = (lambda x, *d: x.transpose(*d))((x @ wq).reshape(B, Sq, Hq, Dh), 0, 2, 1, 3)
        k = jnp.repeat(k_cache[:, :, Sk - W:, :], rep, axis=1)
        v = jnp.repeat(v_cache[:, :, Sk - W:, :], rep, axis=1)
        scores = jnp.einsum("bhqd,bhkd->bhqk", q, k) * (Dh ** -0.5)
        p = _softmax(scores, axis=-1)
        o = jnp.einsum("bhqk,bhkd->bhqd", p, v)
        return (lambda x, *d: x.transpose(*d))(o, 0, 2, 1, 3).reshape(B, Sq, Hq * Dh) @ wo

    def _B_ref(x, w_r, w_gate, w_up, w_down):
        B, S, D = x.shape
        C = 1
        r = x @ w_r
        idx = jnp.argsort(-r, axis=-1)[:, :C]
        idx_e = jnp.repeat(idx.reshape(B, C, 1), D, axis=2)
        x_sel = jnp.take_along_axis(x, idx_e, axis=1)
        g = _silu(x_sel @ w_gate)
        u = x_sel @ w_up
        y = (g * u) @ w_down
        r_sel = _sigmoid(jnp.take_along_axis(r, idx, axis=1))
        y = y * r_sel.reshape(B, C, 1)
        b_off = (jnp.arange(B) * S).reshape(B, 1)
        flat_idx = (idx + b_off).reshape(B * C)
        zero = (x * 0.0).reshape(B * S, D)
        upd = _scatter_add(zero, flat_idx, y.reshape(B * C, D), axis=0)
        return x + upd.reshape(B, S, D)

    x = A_x
    x = x + _A_ref(_layernorm(x, axis=-1), A_k_cache, A_v_cache, A_wq, A_wo)
    x = x + _B_ref(_layernorm(x, axis=-1), B_w_r, B_w_gate, B_w_up, B_w_down)
    x = x + _A_ref(_layernorm(x, axis=-1), A_k_cache, A_v_cache, A_wq, A_wo)
    x = x + _B_ref(_layernorm(x, axis=-1), B_w_r, B_w_gate, B_w_up, B_w_down)
    return x
```

```python
import functools
import math

import jax
import jax.numpy as jnp
import jax.experimental.pallas as pl
import jax.experimental.pallas.tpu as pltpu

B, D, H, DH, SK, F = 4, 640, 32, 192, 4096, 1536
W = 1024
NP = H // 2
PD = 2 * DH
EPS = 1e-5
BF = jnp.bfloat16
F32 = jnp.float32
EXP2_SCALE = (DH ** -0.5) * math.log2(math.e)

V_LAST_CHUNKS = (8, 4, 2, 1, 1)
GROUP = 2


def _layernorm(x):
    m = jnp.mean(x, axis=-1, keepdims=True)
    xc = x - m
    v = jnp.mean(xc * xc, axis=-1, keepdims=True)
    return xc * jax.lax.rsqrt(v + EPS)


def _kernel(x_hbm, kt_hbm, vt_hbm, wq_hbm, wo_hbm, wr_hbm, wg_hbm, wu_hbm, wd_hbm,
            out_ref,
            xin, kbuf, vbuf, wq, wo, wr, wg, wu, wd, xs, sems):
    win = pl.ds(SK - W, W)

    small = [pltpu.make_async_copy(x_hbm, xin, sems.at[0]),
             pltpu.make_async_copy(wr_hbm, wr, sems.at[1])]
    weights = [pltpu.make_async_copy(s, d, sems.at[2 + i]) for i, (s, d) in enumerate(
        [(wq_hbm, wq), (wo_hbm, wo), (wg_hbm, wg), (wu_hbm, wu), (wd_hbm, wd)])]

    def k_copy(b):
        return pltpu.make_async_copy(kt_hbm.at[b, :, :, win], kbuf.at[b], sems.at[7 + b])

    def v_copy(b):
        return pltpu.make_async_copy(vt_hbm.at[b, :, :, win], vbuf.at[b], sems.at[11 + b])

    v_last = []
    start = 0
    for i, n in enumerate(V_LAST_CHUNKS):
        v_last.append((start, pltpu.make_async_copy(
            vt_hbm.at[B - 1, pl.ds(start, n), :, win], vbuf.at[B - 1, pl.ds(start, n)],
            sems.at[14 + i])))
        start += n

    for c in small + weights:
        c.start()
    for b in range(B - 1):
        k_copy(b).start()
        v_copy(b).start()
    k_copy(B - 1).start()
    for _, c in v_last:
        c.start()

    for c in small:
        c.wait()
    x_all = xin[...].astype(F32)
    for b in range(B):
        xs[b] = jnp.broadcast_to(x_all[b:b + 1, :], (8, D))
    for c in weights:
        c.wait()

    lane = jax.lax.broadcasted_iota(jnp.int32, (8, 128), 1)
    sub = jax.lax.broadcasted_iota(jnp.int32, (8, 128), 0)
    lane_pd = jax.lax.broadcasted_iota(jnp.int32, (8, PD), 1)

    def q_proj(g, xn):
        q = jnp.dot(xn, wq[:, g * PD:(g + 1) * PD], preferred_element_type=F32)
        return jnp.concatenate([jnp.where(lane_pd < DH, q, 0.0),
                                jnp.where(lane_pd >= DH, q, 0.0)], axis=0).astype(BF)

    def scores(b, g, qm):
        s = jnp.dot(qm, kbuf[b, g], preferred_element_type=F32)
        mx = jnp.max(s, axis=-1, keepdims=True)
        p = jnp.exp2((s - mx) * EXP2_SCALE)
        inv = 1.0 / jnp.sum(p, axis=-1, keepdims=True)
        return p, inv

    def pv(b, g, p, inv):
        tiles = [jnp.zeros((8, 128), F32) for _ in range(PD // 128)]
        for r in range(PD // 8):
            hh = r // (DH // 8)
            ph = p[8 * hh:8 * hh + 8, :]
            prod = vbuf[b, g, 8 * r:8 * r + 8, :].astype(F32) * ph
            part = prod[:, 0:128]
            for c in range(1, W // 128):
                part = part + prod[:, 128 * c:128 * (c + 1)]
            o_col = jnp.sum(part, axis=-1, keepdims=True)
            t, off = divmod(8 * r, 128)
            tiles[t] = jnp.where(lane == sub + off, o_col, tiles[t])
        o = jnp.concatenate(tiles, axis=1)
        o = o * jnp.where(lane_pd < DH, inv[0:8], inv[8:16])
        return o.astype(BF)

    def o_proj(g, o):
        return jnp.dot(o, wo[g * PD:(g + 1) * PD, :], preferred_element_type=F32)

    def half(j, carry):
        b = j // 2
        first = (j % 2) == 0

        @pl.when(first)
        def _():
            k_copy(b).wait()

        @pl.when(jnp.logical_and(first, b < B - 1))
        def _():
            v_copy(b).wait()

        x = xs[b]
        xn = _layernorm(x).astype(BF)

        waits = dict(v_last)
        qs, ps, os_ = {}, {}, {}
        acc = jnp.zeros((8, D), F32)
        for i in range(-2, NP + 1):
            if 0 <= i + 2 < NP:
                qs[i + 2] = q_proj(i + 2, xn)
            if 0 <= i + 1 < NP:
                ps[i + 1] = scores(b, i + 1, qs.pop(i + 1))
            if 0 <= i - 1 < NP:
                acc = acc + o_proj(i - 1, os_.pop(i - 1))
            if 0 <= i < NP:
                if i in waits:
                    @pl.when(j == 2 * (B - 1))
                    def _():
                        waits[i].wait()
                os_[i] = pv(b, i, *ps.pop(i))
        x1 = x + jnp.sum(acc, axis=0, keepdims=True)

        xn1 = _layernorm(x1)
        wrf = wr[...].astype(F32)
        rp = xn1[:, 0:128] * wrf[0:1, :]
        for t in range(1, D // 128):
            rp = rp + xn1[:, 128 * t:128 * (t + 1)] * wrf[t:t + 1, :]
        r = jnp.sum(rp, axis=-1, keepdims=True)
        xb = xn1.astype(BF)
        gt = jnp.dot(xb, wg[...], preferred_element_type=F32)
        up = jnp.dot(xb, wu[...], preferred_element_type=F32)
        hid = (gt * jax.nn.sigmoid(gt) * up).astype(BF)
        y = jnp.dot(hid, wd[...], preferred_element_type=F32)
        xs[b] = x1 + xn1 + y * jax.nn.sigmoid(r)
        return carry

    jax.lax.fori_loop(0, 2 * B, half, 0)

    sub_d = jax.lax.broadcasted_iota(jnp.int32, (8, D), 0)
    res = xs[0]
    for b in range(1, B):
        res = jnp.where(sub_d == b, xs[b], res)
    out_ref[...] = res[0:B, :].astype(BF)


@jax.jit
def pallas_interleave_layers__sliding_block_cached__moe_arch_mod__decode_kernel(
    A_x: jax.Array,
    A_k_cache: jax.Array,
    A_v_cache: jax.Array,
    A_wq: jax.Array,
    A_wo: jax.Array,
    B_x: jax.Array,
    B_w_r: jax.Array,
    B_w_gate: jax.Array,
    B_w_up: jax.Array,
    B_w_down: jax.Array,
):
    del B_x
    kt = jnp.swapaxes(A_k_cache, 2, 3).reshape(B, NP, PD, SK)
    vt = jnp.swapaxes(A_v_cache, 2, 3).reshape(B, NP, PD, SK)
    n_sems = 14 + len(V_LAST_CHUNKS)
    out = pl.pallas_call(
        _kernel,
        out_shape=jax.ShapeDtypeStruct((B, D), BF),
        in_specs=[pl.BlockSpec(memory_space=pl.ANY)] * 9,
        out_specs=pl.BlockSpec(memory_space=pltpu.VMEM),
        scratch_shapes=[
            pltpu.VMEM((B, D), BF),
            pltpu.VMEM((B, NP, PD, W), BF),
            pltpu.VMEM((B, NP, PD, W), BF),
            pltpu.VMEM((D, H * DH), BF),
            pltpu.VMEM((H * DH, D), BF),
            pltpu.VMEM((D // 128, 128), BF),
            pltpu.VMEM((D, F), BF),
            pltpu.VMEM((D, F), BF),
            pltpu.VMEM((F, D), BF),
            pltpu.VMEM((B, 8, D), F32),
            pltpu.SemaphoreType.DMA((n_sems,)),
        ],
        compiler_params=pltpu.CompilerParams(vmem_limit_bytes=124 * 1024 * 1024),
    )(A_x.reshape(B, D), kt, vt, A_wq, A_wo, B_w_r.reshape(D // 128, 128),
      B_w_gate, B_w_up, B_w_down)
    return out.reshape(B, 1, D)
```

```python
import math

import jax
import jax.numpy as jnp
import jax.experimental.pallas as pl
import jax.experimental.pallas.tpu as pltpu

B, D, H, DH, SK, F = 4, 640, 32, 192, 4096, 1536
W = 1024
NP = H // 2
PD = 2 * DH
EPS = 1e-5
BF = jnp.bfloat16
F32 = jnp.float32
U32 = jnp.uint32
EXP2_SCALE = (DH ** -0.5) * math.log2(math.e)

V_LAST_CHUNKS = (6, 4, 2, 2, 1)
N_SEMS = 14 + len(V_LAST_CHUNKS) + 2
WO_VPU = 256
WO_MXU = PD - WO_VPU
FA = 7
KD = 7
NF = F // 128
STAT = 'one'
LQ = 2
LK = 1


def _dot(a, b):
    return jnp.dot(a, b, preferred_element_type=F32)


def _bf(u):
    return pltpu.bitcast(u, BF)


def _stats(x):
    m = jnp.mean(x, axis=-1, keepdims=True)
    xc = x - m
    v = jnp.mean(xc * xc, axis=-1, keepdims=True)
    return m, jax.lax.rsqrt(v + EPS)


def _fold(x):
    part = x[:, 0:128]
    for c in range(1, x.shape[1] // 128):
        part = part + x[:, 128 * c:128 * (c + 1)]
    return part


def _rowsum(x):
    return jnp.broadcast_to(jnp.sum(x, axis=0, keepdims=True), x.shape)


def _sigmoid(x):
    return 0.5 * jnp.tanh(0.5 * x) + 0.5


def _silu_mul(g, u):
    return g * _sigmoid(g) * u


def _recip(x):
    r = pl.reciprocal(x, approx=True)
    return r * (2.0 - x * r)


def _kernel(x_hbm, kt_hbm, vt_hbm, wq_hbm, wo_hbm, wr_hbm, wg_hbm, wu_hbm, wd_hbm,
            out_ref,
            xin, knat, vnat, wq_n, wo_n, wr, wg_n, wu_n, wd_n,
            ku, vf, wq, wo_u, wo_f, wg, wu, wd, wg_f, wu_f, wd_f,
            csq, csg, csu, xs, accs, ps, sems):
    win = pl.ds(SK - W, W)

    small = [pltpu.make_async_copy(x_hbm, xin, sems.at[0]),
             pltpu.make_async_copy(wr_hbm, wr, sems.at[1])]
    weights = [pltpu.make_async_copy(s, d, sems.at[2 + i]) for i, (s, d) in enumerate(
        [(wq_hbm, wq_n), (wo_hbm, wo_n), (wg_hbm, wg_n), (wu_hbm, wu_n), (wd_hbm, wd_n)])]

    def k_copy(b):
        return pltpu.make_async_copy(kt_hbm.at[b, :, :, win], knat, sems.at[7 + b])

    def v_copy(b):
        return pltpu.make_async_copy(vt_hbm.at[b, :, :, win], vnat, sems.at[11 + b])

    v_last = []
    start = 0
    for i, n in enumerate(V_LAST_CHUNKS):
        v_last.append((start, pltpu.make_async_copy(
            vt_hbm.at[B - 1, pl.ds(start, n), :, win],
            vnat.at[pl.ds(start, n)], sems.at[14 + i])))
        start += n
    v_heads = [pltpu.make_async_copy(
        vt_hbm.at[B - 1, NP - 1, pl.ds(hh * DH, DH), win],
        vnat.at[NP - 1, pl.ds(hh * DH, DH)],
        sems.at[14 + len(V_LAST_CHUNKS) + hh]) for hh in range(2)]

    for c in small + weights:
        c.start()
    k_copy(0).start()
    v_copy(0).start()

    for c in small:
        c.wait()
    x_all = xin[...].astype(F32)
    for b in range(B):
        xs[b] = jnp.broadcast_to(x_all[b:b + 1, :], (8, D))

    def row_loop(n_rows, rows, fn):
        def body(i, c):
            fn(pl.ds(pl.multiple_of(i * rows, 16), rows),
               pl.ds(pl.multiple_of(i * (rows // 2), 8), rows // 2))
            return c
        jax.lax.fori_loop(0, n_rows // rows, body, 0)

    ones = jnp.ones((8, D), BF)
    weights[0].wait()

    def wq_fn(r, r2):
        wq[r2, :] = pltpu.bitcast(wq_n[r, :], U32)
    row_loop(D, 16, wq_fn)

    def csq_body(i, c):
        col = pl.ds(pl.multiple_of(i * 768, 128), 768)
        csq[:, col] = _dot(ones, _bf(wq[:, col]))
        return c
    jax.lax.fori_loop(0, H * DH // 768, csq_body, 0)
    weights[1].wait()

    def wo_body(g, c):
        r = pl.multiple_of(g * PD, 128)
        wo_f[g] = wo_n[pl.ds(r, WO_VPU), :].astype(F32)
        wo_u[g] = pltpu.bitcast(wo_n[pl.ds(r + WO_VPU, WO_MXU), :], U32)
        return c
    jax.lax.fori_loop(0, NP, wo_body, 0)

    for cp, src, dst_u, dst_f, cs in ((weights[2], wg_n, wg, wg_f, csg),
                                      (weights[3], wu_n, wu, wu_f, csu)):
        cp.wait()

        def gu_fn(r, r2, src=src, dst_u=dst_u, dst_f=dst_f):
            dst_u[r2, :] = pltpu.bitcast(src[r, 0:FA * 128], U32)
            dst_f[r, :] = src[r, FA * 128:].astype(F32)
        row_loop(D, 64, gu_fn)
        cs[...] = _dot(ones, src[...])
    weights[4].wait()

    def wdf_fn(r, r2):
        wd_f[r, :] = wd_n[r, :].astype(F32)
    row_loop(KD * 128, 128, wdf_fn)
    wd[...] = pltpu.bitcast(wd_n[KD * 128:, :], U32)

    lane = jax.lax.broadcasted_iota(jnp.int32, (8, 128), 1)
    sub = jax.lax.broadcasted_iota(jnp.int32, (8, 128), 0)
    lane_pd = jax.lax.broadcasted_iota(jnp.int32, (8, PD), 1)

    def cols(g):
        if isinstance(g, int):
            return slice(g * PD, (g + 1) * PD)
        return pl.ds(pl.multiple_of(g * PD, 128), PD)

    def column(x, r):
        t, off = divmod(8 * r, 128)
        return jnp.sum(jnp.where(lane == sub + off, x[:, 128 * t:128 * (t + 1)], 0.0),
                       axis=-1, keepdims=True)

    def q_proj(g, xb, m, rs):
        q = (_dot(xb, _bf(wq[:, cols(g)])) - m * csq[:, cols(g)]) * rs
        return jnp.concatenate([jnp.where(lane_pd < DH, q, 0.0),
                                jnp.where(lane_pd >= DH, q, 0.0)], axis=0).astype(BF)

    def ffn(x1):
        x1b = x1.astype(BF)
        x1 = x1b.astype(F32)
        if STAT == "two":
            m1, rs1 = _stats(x1)
            xc = x1 - m1
            xsrc = x1
        elif STAT == "center":
            m1, rs1 = _stats(x1)
            xc = x1 - m1
            xsrc = xc
        elif STAT == "one":
            both = jnp.concatenate([_fold(x1), _fold(x1 * x1)], axis=0)
            both = jnp.sum(both, axis=-1, keepdims=True) * (1.0 / D)
            m1 = both[0:8]
            rs1 = jax.lax.rsqrt(both[8:16] - m1 * m1 + EPS)
            xc = x1 - m1
            xsrc = x1
        ag = au = None
        for r in range(D // 8):
            c = column(xsrc, r)
            tg = c * wg_f[8 * r:8 * r + 8, :]
            tu = c * wu_f[8 * r:8 * r + 8, :]
            ag = tg if ag is None else ag + tg
            au = tu if au is None else au + tu
        hs = []
        for t in range(FA):
            cs = slice(128 * t, 128 * (t + 1))
            g = (_dot(x1b, _bf(wg[:, cs])) - m1 * csg[:, cs]) * rs1
            u = (_dot(x1b, _bf(wu[:, cs])) - m1 * csu[:, cs]) * rs1
            hs.append(_silu_mul(g, u))
        if STAT == "center":
            hv = _silu_mul(_rowsum(ag) * rs1, _rowsum(au) * rs1)
        else:
            hv = _silu_mul((_rowsum(ag) - m1 * csg[:, FA * 128:]) * rs1,
                           (_rowsum(au) - m1 * csu[:, FA * 128:]) * rs1)
        yv = None
        for t in range(KD):
            for r in range(16):
                tv = column(hs[t], r) * wd_f[128 * t + 8 * r:128 * t + 8 * r + 8, :]
                yv = tv if yv is None else yv + tv
        hm = jnp.concatenate(hs[KD:] + [hv], axis=1).astype(BF)
        ym = None
        for t in range(NF - KD):
            tm = _dot(hm[:, 128 * t:128 * (t + 1)], _bf(wd[64 * t:64 * (t + 1), :]))
            ym = tm if ym is None else ym + tm
        xn1 = xc * rs1
        wrf = wr[...].astype(F32)
        rp = xn1[:, 0:128] * wrf[0:1, :]
        for t in range(1, D // 128):
            rp = rp + xn1[:, 128 * t:128 * (t + 1)] * wrf[t:t + 1, :]
        gate = _sigmoid(jnp.sum(rp, axis=-1, keepdims=True))
        return (x1 + xn1 + (ym + _rowsum(yv)) * gate).astype(BF).astype(F32)

    def attention2(x):
        xb = x.astype(BF)
        m, rs = _stats(x)
        rs = rs * EXP2_SCALE
        qs, mxs, oms = {}, {}, {}
        acc = None
        for i in range(-LQ, NP):
            if 0 <= i + LQ < NP:
                qs[i + LQ] = q_proj(i + LQ, xb, m, rs)
            g = i + LK
            if 0 <= g < NP:
                qm = qs.pop(g)
                run = None
                for c in range(W // 128):
                    sc = _dot(qm, _bf(ku[g, :, c * 128:(c + 1) * 128]))
                    ps[g, :, c * 128:(c + 1) * 128] = sc
                    run = sc if run is None else jnp.maximum(run, sc)
                mxs[g] = jnp.max(run, axis=-1, keepdims=True)
            if 0 <= i < NP:
                tiles = [jnp.zeros((8, 128), F32) for _ in range(WO_MXU // 128)]
                invs = []
                for hh in range(2):
                    ph = jnp.exp2(ps[i, 8 * hh:8 * hh + 8, :] - mxs[i][8 * hh:8 * hh + 8])
                    inv = _recip(jnp.sum(_fold(ph), axis=-1, keepdims=True))
                    invs.append(inv)
                    acc_h = None
                    for r in range(hh * (DH // 8), (hh + 1) * (DH // 8)):
                        o_col = jnp.sum(_fold(vf[i, 8 * r:8 * r + 8, :] * ph),
                                        axis=-1, keepdims=True)
                        if 8 * r < WO_VPU:
                            t = o_col * wo_f[i, 8 * r:8 * r + 8, :]
                            acc_h = t if acc_h is None else acc_h + t
                        else:
                            t, off = divmod(8 * r - WO_VPU, 128)
                            tiles[t] = jnp.where(lane == sub + off, o_col, tiles[t])
                    if acc_h is not None:
                        acc = acc_h * inv if acc is None else acc + acc_h * inv
                o = jnp.concatenate(tiles, axis=1)
                o = o * jnp.where(lane_pd < DH, invs[0], invs[1])[:, WO_VPU:]
                oms[i] = o.astype(BF)
        acc2 = None
        for i in range(NP):
            t = _dot(oms[i], _bf(wo_u[i]))
            acc2 = t if acc2 is None else acc2 + t
        return acc + acc2

    def batch(b, carry):
        last = b == B - 1
        x = xs[b]

        k_copy(b).wait()

        def body_k(i, c):
            g = i // 4
            r = pl.multiple_of((i % 4) * 96, 16)
            ku[g, pl.ds(pl.multiple_of((i % 4) * 48, 8), 48), :] = pltpu.bitcast(
                knat[g, pl.ds(r, 96), :], U32)
            return c
        jax.lax.fori_loop(0, NP * 4, body_k, 0)

        @pl.when(b < B - 1)
        def _():
            k_copy(b + 1).start()

        xb = x.astype(BF)
        m, rs = _stats(x)
        rs = rs * EXP2_SCALE

        def body_a(i, c):
            qs = [q_proj(4 * i + u, xb, m, rs) for u in range(4)]
            for u in range(4):
                s = _dot(qs[u], _bf(ku[4 * i + u]))
                p = jnp.exp2(s - jnp.max(s, axis=-1, keepdims=True))
                ps[4 * i + u] = p * _recip(jnp.sum(p, axis=-1, keepdims=True))
            return c
        jax.lax.fori_loop(0, NP // 4, body_a, 0)

        @pl.when(b < B - 1)
        def _():
            v_copy(b).wait()

        def pv1(g, r0, r1):
            out = []
            for r in range(r0, r1):
                if r == r0 or r % (DH // 8) == 0:
                    hh = r // (DH // 8)
                    ph = ps[g, 8 * hh:8 * hh + 8, :]
                v = vnat[g, 8 * r:8 * r + 8, :].astype(F32)
                vf[g, 8 * r:8 * r + 8, :] = v
                out.append(jnp.sum(_fold(v * ph), axis=-1, keepdims=True))
            return out

        def scatter(o_cols):
            tiles = [jnp.zeros((8, 128), F32) for _ in range((len(o_cols) + 15) // 16)]
            for r, o_col in enumerate(o_cols):
                t, off = divmod(8 * r, 128)
                tiles[t] = jnp.where(lane == sub + off, o_col, tiles[t])
            return jnp.concatenate(tiles, axis=1)[:, :8 * len(o_cols)].astype(BF)

        def o_proj(g, o):
            return _dot(o, wo_n[pl.ds(pl.multiple_of(g * PD, 128), PD), :])

        def body_b(g, c):
            acc, o_prev = c
            for start, cp in v_last:
                @pl.when(jnp.logical_and(last, g == start))
                def _():
                    cp.wait()
            acc = acc + o_proj(jnp.maximum(g - 1, 0), o_prev)
            return acc, scatter(pv1(g, 0, PD // 8))
        acc, o_prev = jax.lax.fori_loop(
            0, NP - 1, body_b, (jnp.zeros((8, D), F32), jnp.zeros((8, PD), BF)))

        @pl.when(last)
        def _():
            v_heads[1].wait()
        acc = acc + o_proj(NP - 2, o_prev)
        acc = acc + _dot(scatter(pv1(NP - 1, DH // 8, PD // 8)), wo_n[H * DH - DH:, :])
        accs[...] = acc

        @pl.when(last)
        def _():
            v_heads[0].wait()
        acc = accs[...]
        for r, o_col in enumerate(pv1(NP - 1, 0, DH // 8)):
            acc = acc + o_col * wo_f[NP - 1, 8 * r:8 * r + 8, :]

        x = ffn(x + _rowsum(acc))
        x = ffn(x + _rowsum(attention2(x)))
        xs[b] = x

        @pl.when(b < B - 2)
        def _():
            v_copy(b + 1).start()

        @pl.when(b == B - 2)
        def _():
            for _, c in v_last:
                c.start()
            v_heads[1].start()
            v_heads[0].start()
        return carry

    jax.lax.fori_loop(0, B, batch, 0)

    sub_d = jax.lax.broadcasted_iota(jnp.int32, (8, D), 0)
    res = xs[0]
    for b in range(1, B):
        res = jnp.where(sub_d == b, xs[b], res)
    out_ref[...] = res[0:B, :].astype(BF)


@jax.jit
def pallas_interleave_layers__sliding_block_cached__moe_arch_mod__decode_kernel(
    A_x: jax.Array,
    A_k_cache: jax.Array,
    A_v_cache: jax.Array,
    A_wq: jax.Array,
    A_wo: jax.Array,
    B_x: jax.Array,
    B_w_r: jax.Array,
    B_w_gate: jax.Array,
    B_w_up: jax.Array,
    B_w_down: jax.Array,
):
    del B_x
    kt = jnp.swapaxes(A_k_cache, 2, 3).reshape(B, NP, PD, SK)
    vt = jnp.swapaxes(A_v_cache, 2, 3).reshape(B, NP, PD, SK)
    out = pl.pallas_call(
        _kernel,
        out_shape=jax.ShapeDtypeStruct((B, D), BF),
        in_specs=[pl.BlockSpec(memory_space=pl.ANY)] * 9,
        out_specs=pl.BlockSpec(memory_space=pltpu.VMEM),
        scratch_shapes=[
            pltpu.VMEM((B, D), BF),
            pltpu.VMEM((NP, PD, W), BF),
            pltpu.VMEM((NP, PD, W), BF),
            pltpu.VMEM((D, H * DH), BF),
            pltpu.VMEM((H * DH, D), BF),
            pltpu.VMEM((D // 128, 128), BF),
            pltpu.VMEM((D, F), BF),
            pltpu.VMEM((D, F), BF),
            pltpu.VMEM((F, D), BF),
            pltpu.VMEM((NP, PD // 2, W), U32),
            pltpu.VMEM((NP, PD, W), F32),
            pltpu.VMEM((D // 2, H * DH), U32),
            pltpu.VMEM((NP, WO_MXU // 2, D), U32),
            pltpu.VMEM((NP, WO_VPU, D), F32),
            pltpu.VMEM((D // 2, FA * 128), U32),
            pltpu.VMEM((D // 2, FA * 128), U32),
            pltpu.VMEM(((NF - KD) * 64, D), U32),
            pltpu.VMEM((D, (NF - FA) * 128), F32),
            pltpu.VMEM((D, (NF - FA) * 128), F32),
            pltpu.VMEM((KD * 128, D), F32),
            pltpu.VMEM((8, H * DH), F32),
            pltpu.VMEM((8, F), F32),
            pltpu.VMEM((8, F), F32),
            pltpu.VMEM((B, 8, D), F32),
            pltpu.VMEM((8, D), F32),
            pltpu.VMEM((NP, 16, W), F32),
            pltpu.SemaphoreType.DMA((N_SEMS,)),
        ],
        compiler_params=pltpu.CompilerParams(vmem_limit_bytes=122 * 1024 * 1024, disable_semaphore_checks=True),
    )(A_x.reshape(B, D), kt, vt, A_wq, A_wo, B_w_r.reshape(D // 128, 128),
      B_w_gate, B_w_up, B_w_down)
    return out.reshape(B, 1, D)
```

```python
import math

import jax
import jax.numpy as jnp
import jax.experimental.pallas as pl
import jax.experimental.pallas.tpu as pltpu

B, D, H, DH, SK, F = 4, 640, 32, 192, 4096, 1536
W = 1024
NP = H // 2
PD = 2 * DH
EPS = 1e-5
BF = jnp.bfloat16
F32 = jnp.float32
U32 = jnp.uint32
EXP2_SCALE = (DH ** -0.5) * math.log2(math.e)

RG = 16
NG = PD // RG
SEM_K = 7
SEM_V = 8
N_SEMS = SEM_V + NG + 1
WO_VPU = 256
WO_MXU = PD - WO_VPU
FA = 7
KD = 7
NF = F // 128
STAT = 'one'
LQ = 2
LK = 1


def _dot(a, b):
    return jnp.dot(a, b, preferred_element_type=F32)


def _bf(u):
    return pltpu.bitcast(u, BF)


def _stats(x):
    m = jnp.mean(x, axis=-1, keepdims=True)
    xc = x - m
    v = jnp.mean(xc * xc, axis=-1, keepdims=True)
    return m, jax.lax.rsqrt(v + EPS)


def _fold(x):
    part = x[:, 0:128]
    for c in range(1, x.shape[1] // 128):
        part = part + x[:, 128 * c:128 * (c + 1)]
    return part


def _rowsum(x):
    return jnp.broadcast_to(jnp.sum(x, axis=0, keepdims=True), x.shape)


def _sigmoid(x):
    return 0.5 * jnp.tanh(0.5 * x) + 0.5


def _silu_mul(g, u):
    return g * _sigmoid(g) * u


def _recip(x):
    r = pl.reciprocal(x, approx=True)
    return r * (2.0 - x * r)


def _kernel(x_hbm, kt_hbm, vt_hbm, wq_hbm, wo_hbm, wr_hbm, wg_hbm, wu_hbm, wd_hbm,
            out_ref,
            xin, knat, vnat, wq_n, wo_n, wr, wg_n, wu_n, wd_n,
            ku, vf, wq, wo_u, wo_f, wg, wu, wd, wg_f, wu_f, wd_f,
            csq, csg, csu, xs, accs, ps, sems):
    win = pl.ds(SK - W, W)

    small = [pltpu.make_async_copy(x_hbm, xin, sems.at[0]),
             pltpu.make_async_copy(wr_hbm, wr, sems.at[1])]
    weights = [pltpu.make_async_copy(s, d, sems.at[2 + i]) for i, (s, d) in enumerate(
        [(wq_hbm, wq_n), (wo_hbm, wo_n), (wg_hbm, wg_n), (wu_hbm, wu_n), (wd_hbm, wd_n)])]

    def rows_copy(src, dst, b, r, n, sem):
        return pltpu.make_async_copy(src.at[b, :, pl.ds(r, n), win], dst.at[:, pl.ds(r, n)],
                                     sems.at[sem])

    def k_start(b):
        def body(j, c):
            rows_copy(kt_hbm, knat, b, pl.multiple_of(j * RG, RG), RG, SEM_K).start()
            return c
        jax.lax.fori_loop(0, NG, body, 0)

    def k_wait():
        pltpu.make_async_copy(knat, knat, sems.at[SEM_K]).wait()

    def v_group(b, j):
        return rows_copy(vt_hbm, vnat, b, pl.multiple_of(j * RG, RG), RG, SEM_V + j)

    def v_half(b, h):
        return rows_copy(vt_hbm, vnat, b, h * (RG // 2), RG // 2, SEM_V + h * NG)

    def v_start(b):
        def body(i, c):
            v_group(b, NG - 1 - i).start()
            return c
        jax.lax.fori_loop(0, NG - 1, body, 0)
        v_half(b, 1).start()
        v_half(b, 0).start()

    for c in small + weights:
        c.start()
    k_start(0)
    v_start(0)

    for c in small:
        c.wait()
    x_all = xin[...].astype(F32)
    for b in range(B):
        xs[b] = jnp.broadcast_to(x_all[b:b + 1, :], (8, D))

    def row_loop(n_rows, rows, fn):
        def body(i, c):
            fn(pl.ds(pl.multiple_of(i * rows, 16), rows),
               pl.ds(pl.multiple_of(i * (rows // 2), 8), rows // 2))
            return c
        jax.lax.fori_loop(0, n_rows // rows, body, 0)

    ones = jnp.ones((8, D), BF)
    weights[0].wait()

    def wq_fn(r, r2):
        wq[r2, :] = pltpu.bitcast(wq_n[r, :], U32)
    row_loop(D, 16, wq_fn)

    def csq_body(i, c):
        col = pl.ds(pl.multiple_of(i * 768, 128), 768)
        csq[:, col] = _dot(ones, _bf(wq[:, col]))
        return c
    jax.lax.fori_loop(0, H * DH // 768, csq_body, 0)
    weights[1].wait()

    def wo_body(g, c):
        wo_f[g] = wo_n[g, 0:WO_VPU, :].astype(F32)
        wo_u[g] = pltpu.bitcast(wo_n[g, WO_VPU:, :], U32)
        return c
    jax.lax.fori_loop(0, NP, wo_body, 0)

    for cp, src, dst_u, dst_f, cs in ((weights[2], wg_n, wg, wg_f, csg),
                                      (weights[3], wu_n, wu, wu_f, csu)):
        cp.wait()

        def gu_fn(r, r2, src=src, dst_u=dst_u, dst_f=dst_f):
            dst_u[r2, :] = pltpu.bitcast(src[r, 0:FA * 128], U32)
            dst_f[r, :] = src[r, FA * 128:].astype(F32)
        row_loop(D, 64, gu_fn)
        cs[...] = _dot(ones, src[...])
    weights[4].wait()

    def wdf_fn(r, r2):
        wd_f[r, :] = wd_n[r, :].astype(F32)
    row_loop(KD * 128, 128, wdf_fn)
    wd[...] = pltpu.bitcast(wd_n[KD * 128:, :], U32)

    lane = jax.lax.broadcasted_iota(jnp.int32, (8, 128), 1)
    sub = jax.lax.broadcasted_iota(jnp.int32, (8, 128), 0)
    lane_pd = jax.lax.broadcasted_iota(jnp.int32, (8, PD), 1)

    def cols(g):
        if isinstance(g, int):
            return slice(g * PD, (g + 1) * PD)
        return pl.ds(pl.multiple_of(g * PD, 128), PD)

    def column(x, r):
        t, off = divmod(8 * r, 128)
        return jnp.sum(jnp.where(lane == sub + off, x[:, 128 * t:128 * (t + 1)], 0.0),
                       axis=-1, keepdims=True)

    def q_proj(g, xb, m, rs):
        q = (_dot(xb, _bf(wq[:, cols(g)])) - m * csq[:, cols(g)]) * rs
        return jnp.concatenate([jnp.where(lane_pd < DH, q, 0.0),
                                jnp.where(lane_pd >= DH, q, 0.0)], axis=0).astype(BF)

    def ffn(x1):
        x1b = x1.astype(BF)
        x1 = x1b.astype(F32)
        if STAT == "two":
            m1, rs1 = _stats(x1)
            xc = x1 - m1
            xsrc = x1
        elif STAT == "center":
            m1, rs1 = _stats(x1)
            xc = x1 - m1
            xsrc = xc
        elif STAT == "one":
            both = jnp.concatenate([_fold(x1), _fold(x1 * x1)], axis=0)
            both = jnp.sum(both, axis=-1, keepdims=True) * (1.0 / D)
            m1 = both[0:8]
            rs1 = jax.lax.rsqrt(both[8:16] - m1 * m1 + EPS)
            xc = x1 - m1
            xsrc = x1
        ag = au = None
        for r in range(D // 8):
            c = column(xsrc, r)
            tg = c * wg_f[8 * r:8 * r + 8, :]
            tu = c * wu_f[8 * r:8 * r + 8, :]
            ag = tg if ag is None else ag + tg
            au = tu if au is None else au + tu
        hs = []
        for t in range(FA):
            cs = slice(128 * t, 128 * (t + 1))
            g = (_dot(x1b, _bf(wg[:, cs])) - m1 * csg[:, cs]) * rs1
            u = (_dot(x1b, _bf(wu[:, cs])) - m1 * csu[:, cs]) * rs1
            hs.append(_silu_mul(g, u))
        if STAT == "center":
            hv = _silu_mul(_rowsum(ag) * rs1, _rowsum(au) * rs1)
        else:
            hv = _silu_mul((_rowsum(ag) - m1 * csg[:, FA * 128:]) * rs1,
                           (_rowsum(au) - m1 * csu[:, FA * 128:]) * rs1)
        yv = None
        for t in range(KD):
            for r in range(16):
                tv = column(hs[t], r) * wd_f[128 * t + 8 * r:128 * t + 8 * r + 8, :]
                yv = tv if yv is None else yv + tv
        hm = jnp.concatenate(hs[KD:] + [hv], axis=1).astype(BF)
        ym = None
        for t in range(NF - KD):
            tm = _dot(hm[:, 128 * t:128 * (t + 1)], _bf(wd[64 * t:64 * (t + 1), :]))
            ym = tm if ym is None else ym + tm
        xn1 = xc * rs1
        wrf = wr[...].astype(F32)
        rp = xn1[:, 0:128] * wrf[0:1, :]
        for t in range(1, D // 128):
            rp = rp + xn1[:, 128 * t:128 * (t + 1)] * wrf[t:t + 1, :]
        gate = _sigmoid(jnp.sum(rp, axis=-1, keepdims=True))
        return (x1 + xn1 + (ym + _rowsum(yv)) * gate).astype(BF).astype(F32)

    def attention2(x):
        xb = x.astype(BF)
        m, rs = _stats(x)
        rs = rs * EXP2_SCALE
        qs, mxs, oms = {}, {}, {}
        acc = None
        for i in range(-LQ, NP):
            if 0 <= i + LQ < NP:
                qs[i + LQ] = q_proj(i + LQ, xb, m, rs)
            g = i + LK
            if 0 <= g < NP:
                qm = qs.pop(g)
                run = None
                for c in range(W // 128):
                    sc = _dot(qm, _bf(ku[g, :, c * 128:(c + 1) * 128]))
                    ps[g, :, c * 128:(c + 1) * 128] = sc
                    run = sc if run is None else jnp.maximum(run, sc)
                mxs[g] = jnp.max(run, axis=-1, keepdims=True)
            if 0 <= i < NP:
                tiles = [jnp.zeros((8, 128), F32) for _ in range(WO_MXU // 128)]
                invs = []
                for hh in range(2):
                    ph = jnp.exp2(ps[i, 8 * hh:8 * hh + 8, :] - mxs[i][8 * hh:8 * hh + 8])
                    inv = _recip(jnp.sum(_fold(ph), axis=-1, keepdims=True))
                    invs.append(inv)
                    acc_h = None
                    for r in range(hh * (DH // 8), (hh + 1) * (DH // 8)):
                        o_col = jnp.sum(_fold(vf[i, 8 * r:8 * r + 8, :] * ph),
                                        axis=-1, keepdims=True)
                        if 8 * r < WO_VPU:
                            t = o_col * wo_f[i, 8 * r:8 * r + 8, :]
                            acc_h = t if acc_h is None else acc_h + t
                        else:
                            t, off = divmod(8 * r - WO_VPU, 128)
                            tiles[t] = jnp.where(lane == sub + off, o_col, tiles[t])
                    if acc_h is not None:
                        acc = acc_h * inv if acc is None else acc + acc_h * inv
                o = jnp.concatenate(tiles, axis=1)
                o = o * jnp.where(lane_pd < DH, invs[0], invs[1])[:, WO_VPU:]
                oms[i] = o.astype(BF)
        acc2 = None
        for i in range(NP):
            t = _dot(oms[i], _bf(wo_u[i]))
            acc2 = t if acc2 is None else acc2 + t
        return acc + acc2

    def batch(b, carry):
        x = xs[b]

        k_wait()

        def body_k(i, c):
            g = i // 4
            r = pl.multiple_of((i % 4) * 96, 16)
            ku[g, pl.ds(pl.multiple_of((i % 4) * 48, 8), 48), :] = pltpu.bitcast(
                knat[g, pl.ds(r, 96), :], U32)
            return c
        jax.lax.fori_loop(0, NP * 4, body_k, 0)

        @pl.when(b < B - 1)
        def _():
            k_start(b + 1)

        xb = x.astype(BF)
        m, rs = _stats(x)
        rs = rs * EXP2_SCALE

        def body_a(i, c):
            qs = [q_proj(4 * i + u, xb, m, rs) for u in range(4)]
            for u in range(4):
                s = _dot(qs[u], _bf(ku[4 * i + u]))
                p = jnp.exp2(s - jnp.max(s, axis=-1, keepdims=True))
                ps[4 * i + u] = p * _recip(jnp.sum(p, axis=-1, keepdims=True))
            return c
        jax.lax.fori_loop(0, NP // 4, body_a, 0)

        def pv1(row0, n_tiles, hrow):
            out = []
            for g in range(NP):
                ph = ps[g, pl.ds(hrow, 8), :]
                for t in range(n_tiles):
                    rows = pl.ds(row0 + 8 * t, 8)
                    v = vnat[g, rows, :].astype(F32)
                    vf[g, rows, :] = v
                    out.append(jnp.sum(_fold(v * ph), axis=-1, keepdims=True))
            return out

        def scatter(o_cols):
            tiles = [jnp.zeros((8, 128), F32) for _ in range(len(o_cols) // 16)]
            for r, o_col in enumerate(o_cols):
                t, off = divmod(8 * r, 128)
                tiles[t] = jnp.where(lane == sub + off, o_col, tiles[t])
            return jnp.concatenate(tiles, axis=1).astype(BF)

        def o_proj(j, o):
            w = wo_n[:, pl.ds(pl.multiple_of(j * RG, RG), RG), :]
            return _dot(o, w.reshape(NP * RG, D))

        def body_b(i, c):
            acc, o_prev = c
            j = NG - 1 - i
            v_group(b, j).wait()
            acc = acc + o_proj(jnp.minimum(j + 1, NG - 1), o_prev)
            hrow = pl.multiple_of(jnp.where(j * RG >= DH, 8, 0), 8)
            return acc, scatter(pv1(pl.multiple_of(j * RG, RG), RG // 8, hrow))
        acc, o_prev = jax.lax.fori_loop(
            0, NG - 1, body_b, (jnp.zeros((8, D), F32), jnp.zeros((8, NP * RG), BF)))

        for h in (1, 0):
            v_half(b, h).wait()
            if h == 1:
                acc = acc + o_proj(1, o_prev)
            else:
                acc = accs[...]
            n_t = RG // 16
            for i, o_col in enumerate(pv1(h * (RG // 2), n_t, 0)):
                r0 = h * (RG // 2) + 8 * (i % n_t)
                acc = acc + o_col * wo_f[i // n_t, r0:r0 + 8, :]
            if h == 1:
                accs[...] = acc

        x = ffn(x + _rowsum(acc))
        x = ffn(x + _rowsum(attention2(x)))
        xs[b] = x

        @pl.when(b < B - 1)
        def _():
            v_start(b + 1)
        return carry

    jax.lax.fori_loop(0, B, batch, 0)

    sub_d = jax.lax.broadcasted_iota(jnp.int32, (8, D), 0)
    res = xs[0]
    for b in range(1, B):
        res = jnp.where(sub_d == b, xs[b], res)
    out_ref[...] = res[0:B, :].astype(BF)


@jax.jit
def pallas_interleave_layers__sliding_block_cached__moe_arch_mod__decode_kernel(
    A_x: jax.Array,
    A_k_cache: jax.Array,
    A_v_cache: jax.Array,
    A_wq: jax.Array,
    A_wo: jax.Array,
    B_x: jax.Array,
    B_w_r: jax.Array,
    B_w_gate: jax.Array,
    B_w_up: jax.Array,
    B_w_down: jax.Array,
):
    del B_x
    kt = jnp.swapaxes(A_k_cache, 2, 3).reshape(B, NP, PD, SK)
    vt = jnp.swapaxes(A_v_cache, 2, 3).reshape(B, NP, PD, SK)
    out = pl.pallas_call(
        _kernel,
        out_shape=jax.ShapeDtypeStruct((B, D), BF),
        in_specs=[pl.BlockSpec(memory_space=pl.ANY)] * 9,
        out_specs=pl.BlockSpec(memory_space=pltpu.VMEM),
        scratch_shapes=[
            pltpu.VMEM((B, D), BF),
            pltpu.VMEM((NP, PD, W), BF),
            pltpu.VMEM((NP, PD, W), BF),
            pltpu.VMEM((D, H * DH), BF),
            pltpu.VMEM((NP, PD, D), BF),
            pltpu.VMEM((D // 128, 128), BF),
            pltpu.VMEM((D, F), BF),
            pltpu.VMEM((D, F), BF),
            pltpu.VMEM((F, D), BF),
            pltpu.VMEM((NP, PD // 2, W), U32),
            pltpu.VMEM((NP, PD, W), F32),
            pltpu.VMEM((D // 2, H * DH), U32),
            pltpu.VMEM((NP, WO_MXU // 2, D), U32),
            pltpu.VMEM((NP, WO_VPU, D), F32),
            pltpu.VMEM((D // 2, FA * 128), U32),
            pltpu.VMEM((D // 2, FA * 128), U32),
            pltpu.VMEM(((NF - KD) * 64, D), U32),
            pltpu.VMEM((D, (NF - FA) * 128), F32),
            pltpu.VMEM((D, (NF - FA) * 128), F32),
            pltpu.VMEM((KD * 128, D), F32),
            pltpu.VMEM((8, H * DH), F32),
            pltpu.VMEM((8, F), F32),
            pltpu.VMEM((8, F), F32),
            pltpu.VMEM((B, 8, D), F32),
            pltpu.VMEM((8, D), F32),
            pltpu.VMEM((NP, 16, W), F32),
            pltpu.SemaphoreType.DMA((N_SEMS,)),
        ],
        compiler_params=pltpu.CompilerParams(vmem_limit_bytes=122 * 1024 * 1024, disable_semaphore_checks=True),
    )(A_x.reshape(B, D), kt, vt, A_wq, A_wo.reshape(NP, PD, D), B_w_r.reshape(D // 128, 128),
      B_w_gate, B_w_up, B_w_down)
    return out.reshape(B, 1, D)
```

```python
import math

import jax
import jax.numpy as jnp
import jax.experimental.pallas as pl
import jax.experimental.pallas.tpu as pltpu

B, D, H, DH, SK, F = 4, 640, 32, 192, 4096, 1536
W = 1024
NP = H // 2
PD = 2 * DH
NF = F // 128
EPS = 1e-5
BF = jnp.bfloat16
F32 = jnp.float32
U32 = jnp.uint32
EXP2_SCALE = (DH ** -0.5) * math.log2(math.e)

RG = 16
NG = PD // RG
LAST = (8, 8)
SEM_K = 7
SEM_V = 8
N_SEMS = SEM_V + NG - 1 + len(LAST)
WO_VPU = 256
WO_MXU = PD - WO_VPU
FA = 7
KD = 7
QS = 2
QR = (2, 2)
QV = sum(QR)


def _dot(a, b):
    return jnp.dot(a, b, preferred_element_type=F32)


def _bf(u):
    return pltpu.bitcast(u, BF)


def _fold(x):
    part = x[:, 0:128]
    for c in range(1, x.shape[1] // 128):
        part = part + x[:, 128 * c:128 * (c + 1)]
    return part


def _rowsum(x):
    return jnp.broadcast_to(jnp.sum(x, axis=0, keepdims=True), x.shape)


def _stats(x, shift):
    d = x - shift
    sq = _fold(d * d)
    both = jnp.concatenate([_fold(d), sq], axis=0)
    both = jnp.sum(both, axis=-1, keepdims=True) * (1.0 / D)
    md = both[0:8]
    var = jnp.maximum(both[8:16] - md * md, 0.0)
    return shift + md, jax.lax.rsqrt(var + EPS), sq


def _after(x, dep):
    return jnp.maximum(x, jnp.minimum(dep, x))


def _sigmoid(x):
    return 0.5 * jnp.tanh(0.5 * x) + 0.5


def _silu_mul(g, u):
    return g * _sigmoid(g) * u


def _recip(x):
    r = pl.reciprocal(x, approx=True)
    return r * (2.0 - x * r)


def _kernel(x_hbm, kt_hbm, vt_hbm, wq_hbm, wo_hbm, wr_hbm, wg_hbm, wu_hbm, wd_hbm,
            out_ref,
            xin, knat, vnat, wq_n, wo_n, wr, wg_n, wu_n, wd_n,
            ku, vf, wq, wo_u, wo_f, wg, wu, wd, wg_f, wu_f, wd_f,
            csq, csg, csu, xs, res, ps, wq_f, sems):
    win = pl.ds(SK - W, W)

    small = [pltpu.make_async_copy(x_hbm, xin, sems.at[0]),
             pltpu.make_async_copy(wr_hbm, wr, sems.at[1])]
    weights = [pltpu.make_async_copy(s, d, sems.at[2 + i]) for i, (s, d) in enumerate(
        [(wq_hbm, wq_n), (wo_hbm, wo_n), (wg_hbm, wg_n), (wu_hbm, wu_n), (wd_hbm, wd_n)])]

    def group_rows(j):
        return pl.ds(pl.multiple_of(j * RG, RG), RG)

    def k_start(b):
        def body(j, c):
            pltpu.make_async_copy(kt_hbm.at[b, :, group_rows(j), win],
                                  knat.at[:, group_rows(j)], sems.at[SEM_K]).start()
            return c
        jax.lax.fori_loop(0, NG, body, 0)

    def k_wait():
        pltpu.make_async_copy(knat, knat, sems.at[SEM_K]).wait()

    def v_group(b, j):
        return pltpu.make_async_copy(vt_hbm.at[b, :, group_rows(j), win],
                                     vnat.at[:, group_rows(j)], sems.at[SEM_V + j - 1])

    def v_piece(b, i):
        pairs = pl.ds(sum(LAST[:i]), LAST[i])
        return pltpu.make_async_copy(vt_hbm.at[b, pairs, pl.ds(0, RG), win],
                                     vnat.at[pairs, pl.ds(0, RG)],
                                     sems.at[SEM_V + NG - 1 + i])

    def v_start(b):
        def body(i, c):
            v_group(b, NG - 1 - i).start()
            return c
        jax.lax.fori_loop(0, NG - 1, body, 0)
        for i in range(len(LAST)):
            v_piece(b, i).start()

    for c in weights[:1] + small + weights[1:]:
        c.start()
    k_start(0)
    v_start(0)

    def row_loop(n_rows, rows, fn):
        def body(i, c):
            fn(pl.ds(pl.multiple_of(i * rows, 16), rows),
               pl.ds(pl.multiple_of(i * (rows // 2), 8), rows // 2))
            return c
        jax.lax.fori_loop(0, n_rows // rows, body, 0)

    ones = jnp.ones((8, D), BF)
    weights[0].wait()

    def wq_fn(r, r2):
        wq[r2, :] = pltpu.bitcast(wq_n[r, :], U32)
        wq_f[r, :] = wq_n[r, QS * PD:(QS + QV) * PD].astype(F32)
    row_loop(D, 16, wq_fn)

    def csq_body(i, c):
        col = pl.ds(pl.multiple_of(i * 768, 128), 768)
        csq[:, col] = _dot(ones, _bf(wq[:, col]))
        return c
    jax.lax.fori_loop(0, H * DH // 768, csq_body, 0)

    for c in small:
        c.wait()
    x_all = xin[...].astype(F32)
    for b in range(B):
        xs[b] = jnp.broadcast_to(x_all[b:b + 1, :], (8, D))
    res[...] = jnp.zeros((8, D), F32)
    weights[1].wait()

    def wo_body(g, c):
        wo_f[g] = wo_n[g, 0:WO_VPU, :].astype(F32)
        wo_u[g] = pltpu.bitcast(wo_n[g, WO_VPU:, :], U32)
        return c
    jax.lax.fori_loop(0, NP, wo_body, 0)

    for cp, src, dst_u, dst_f, cs in ((weights[2], wg_n, wg, wg_f, csg),
                                      (weights[3], wu_n, wu, wu_f, csu)):
        cp.wait()

        def gu_fn(r, r2, src=src, dst_u=dst_u, dst_f=dst_f):
            dst_u[r2, :] = pltpu.bitcast(src[r, 0:FA * 128], U32)
            dst_f[r, :] = src[r, FA * 128:].astype(F32)
        row_loop(D, 64, gu_fn)
        cs[...] = _dot(ones, src[...])
    weights[4].wait()

    def wdf_fn(r, r2):
        wd_f[r, :] = wd_n[r, :].astype(F32)
    row_loop(KD * 128, 128, wdf_fn)
    wd[...] = pltpu.bitcast(wd_n[KD * 128:, :], U32)

    lane = jax.lax.broadcasted_iota(jnp.int32, (8, 128), 1)
    sub = jax.lax.broadcasted_iota(jnp.int32, (8, 128), 0)
    lane_pd = jax.lax.broadcasted_iota(jnp.int32, (8, PD), 1)
    sub_d = jax.lax.broadcasted_iota(jnp.int32, (8, D), 0)

    def cols(g):
        if isinstance(g, int):
            return slice(g * PD, (g + 1) * PD)
        return pl.ds(pl.multiple_of(g * PD, 128), PD)

    def column(x, r, how=0):
        t, off = divmod(8 * r, 128)
        xt = x[:, 128 * t:128 * (t + 1)]
        red, fill = ((jnp.sum, 0.0), (jnp.max, -jnp.inf), (jnp.min, jnp.inf))[how]
        return red(jnp.where(lane == sub + off, xt, fill), axis=-1, keepdims=True)

    def matvec(x, w_ref, n_rows, cs=slice(None), how=0):
        acc = None
        for r in range(n_rows // 8):
            t = column(x, r, how) * w_ref[8 * r:8 * r + 8, cs]
            acc = t if acc is None else acc + t
        return acc

    def scatter(o_cols):
        tiles = [jnp.zeros((8, 128), F32) for _ in range(len(o_cols) // 16)]
        for r, o_col in enumerate(o_cols):
            t, off = divmod(8 * r, 128)
            tiles[t] = jnp.where(lane == sub + off, o_col, tiles[t])
        return jnp.concatenate(tiles, axis=1)

    def split_heads(q):
        return jnp.concatenate([jnp.where(lane_pd < DH, q, 0.0),
                                jnp.where(lane_pd >= DH, q, 0.0)], axis=0).astype(BF)

    def q_proj(g, xb, m, rs):
        return split_heads((_dot(xb, _bf(wq[:, cols(g)])) - m * csq[:, cols(g)]) * rs)

    def ffn(x1, shift):
        x1b = x1.astype(BF)
        x1 = x1b.astype(F32)
        m1, rs1, sq = _stats(x1, shift)
        xv = _after(x1, jnp.concatenate([sq] * (D // 128), axis=1))
        ag = matvec(xv, wg_f, D)
        au = matvec(xv, wu_f, D, how=1)
        hs = []
        for t in range(FA):
            cs = slice(128 * t, 128 * (t + 1))
            g = (_dot(x1b, _bf(wg[:, cs])) - m1 * csg[:, cs]) * rs1
            u = (_dot(x1b, _bf(wu[:, cs])) - m1 * csu[:, cs]) * rs1
            hs.append(_silu_mul(g, u))
        hv = _silu_mul((_rowsum(ag) - m1 * csg[:, FA * 128:]) * rs1,
                       (_rowsum(au) - m1 * csu[:, FA * 128:]) * rs1)
        yv = matvec(jnp.concatenate(hs[:KD], axis=1), wd_f, KD * 128)
        hm = jnp.concatenate(hs[KD:] + [hv], axis=1).astype(BF)
        ym = None
        for t in range(NF - KD):
            tm = _dot(hm[:, 128 * t:128 * (t + 1)], _bf(wd[64 * t:64 * (t + 1), :]))
            ym = tm if ym is None else ym + tm
        xn1 = (x1 - m1) * rs1
        wrf = wr[...].astype(F32)
        rp = xn1[:, 0:128] * wrf[0:1, :]
        for t in range(1, D // 128):
            rp = rp + xn1[:, 128 * t:128 * (t + 1)] * wrf[t:t + 1, :]
        gate = _sigmoid(jnp.sum(rp, axis=-1, keepdims=True))
        return x1 + xn1 + (ym + _rowsum(yv)) * gate, m1

    def attention2(x, shift):
        xb = x.astype(BF)
        m, rs, _ = _stats(x, shift)
        rs = rs * EXP2_SCALE
        qs, mxs, runs, oms = {}, {}, {}, []
        for k, n in enumerate(QR):
            u0 = sum(QR[:k])
            qv = _rowsum(matvec(x, wq_f, D, slice(u0 * PD, (u0 + n) * PD), k))
            qv = (qv - m * csq[:, (QS + u0) * PD:(QS + u0 + n) * PD]) * rs
            for u in range(n):
                qs[QS + u0 + u] = split_heads(qv[:, u * PD:(u + 1) * PD])
        acc = None
        for i in range(-2, NP):
            if i + 2 < NP and i + 2 not in qs:
                qs[i + 2] = q_proj(i + 2, xb, m, rs)
            g = i + 1
            if 0 <= g < NP:
                run = None
                for c in range(W // 128):
                    cs = slice(c * 128, (c + 1) * 128)
                    d = [_dot(qs[g][:, 128 * k:128 * (k + 1)],
                              _bf(ku[g, 64 * k:64 * (k + 1), cs])) for k in range(3)]
                    sc = jnp.concatenate([d[0][0:8] + d[1][0:8], d[1][8:16] + d[2][8:16]],
                                         axis=0)
                    ps[g, :, cs] = sc
                    run = sc if run is None else jnp.maximum(run, sc)
                mxs[g] = jnp.max(run, axis=-1, keepdims=True)
                runs[g] = run
            if i >= 0:
                rest = []
                for hh in range(2):
                    mx = mxs[i][8 * hh:8 * hh + 8]
                    if i + 1 < NP:
                        mx = jnp.concatenate([_after(mx, runs[i + 1][0:8])] * (W // 128), axis=1)
                    ph = jnp.exp2(ps[i, 8 * hh:8 * hh + 8, :] - mx)
                    inv = _recip(jnp.sum(_fold(ph), axis=-1, keepdims=True))
                    acc_h = None
                    for r in range(hh * (DH // 8), (hh + 1) * (DH // 8)):
                        o_col = jnp.sum(_fold(vf[i, 8 * r:8 * r + 8, :] * ph),
                                        axis=-1, keepdims=True)
                        if 8 * r < WO_VPU:
                            t = o_col * wo_f[i, 8 * r:8 * r + 8, :]
                            acc_h = t if acc_h is None else acc_h + t
                        else:
                            rest.append(o_col)
                    acc = acc_h * inv if acc is None else acc + acc_h * inv
                    if hh == 1:
                        oms.append((scatter(rest) * inv).astype(BF))
        acc2 = None
        for i in range(NP):
            t = _dot(oms[i], _bf(wo_u[i]))
            acc2 = t if acc2 is None else acc2 + t
        return acc + acc2, m

    def batch(b, carry):
        x = xs[b]

        k_wait()

        def body_k(i, c):
            g = i // 4
            r = pl.multiple_of((i % 4) * 96, 16)
            ku[g, pl.ds(pl.multiple_of((i % 4) * 48, 8), 48), :] = pltpu.bitcast(
                knat[g, pl.ds(r, 96), :], U32)
            return c
        jax.lax.fori_loop(0, NP * 4, body_k, 0)

        @pl.when(b < B - 1)
        def _():
            k_start(b + 1)

        xb = x.astype(BF)
        m, rs, _ = _stats(x, jnp.mean(x, axis=-1, keepdims=True))
        rs = rs * EXP2_SCALE

        def body_a(i, c):
            qs = [q_proj(4 * i + u, xb, m, rs) for u in range(4)]
            for u in range(4):
                s = _dot(qs[u], _bf(ku[4 * i + u]))
                p = jnp.exp2(s - jnp.max(s, axis=-1, keepdims=True))
                ps[4 * i + u] = p * _recip(jnp.sum(p, axis=-1, keepdims=True))
            return c
        jax.lax.fori_loop(0, NP // 4, body_a, 0)

        def pv1(pairs, row0, hrow):
            out = []
            for g in pairs:
                ph = ps[g, pl.ds(hrow, 8), :]
                for t in range(RG // 8):
                    rows = pl.ds(row0 + 8 * t, 8)
                    v = vnat[g, rows, :].astype(F32)
                    vf[g, rows, :] = v
                    out.append(jnp.sum(_fold(v * ph), axis=-1, keepdims=True))
            return out

        def o_proj(j, o):
            return _dot(o, wo_n[:, group_rows(j), :].reshape(NP * RG, D))

        def body_b(i, c):
            acc, o_prev = c
            j = NG - 1 - i
            v_group(b, j).wait()
            acc = acc + o_proj(jnp.minimum(j + 1, NG - 1), o_prev)
            hrow = pl.multiple_of(jnp.where(j * RG >= DH, 8, 0), 8)
            o_cols = pv1(range(NP), pl.multiple_of(j * RG, RG), hrow)
            return acc, scatter(o_cols).astype(BF)
        acc, o_prev = jax.lax.fori_loop(
            0, NG - 1, body_b, (jnp.zeros((8, D), F32), jnp.zeros((8, NP * RG), BF)))

        for i in range(len(LAST)):
            v_piece(b, i).wait()
            if i == 0:
                acc = acc + o_proj(1, o_prev)
            g0 = sum(LAST[:i])
            for k, o_col in enumerate(pv1(range(g0, g0 + LAST[i]), 0, 0)):
                g, t = divmod(k, RG // 8)
                acc = acc + o_col * wo_f[g0 + g, 8 * t:8 * t + 8, :]

        x, m = ffn(x + _rowsum(acc), m)
        x = x.astype(BF).astype(F32)
        acc, m = attention2(x, m)
        x, _ = ffn(x + _rowsum(acc), m)
        r = jnp.where(sub_d == b, x, res[...])
        res[...] = r
        out_ref[...] = r[0:B, :].astype(BF)

        @pl.when(b < B - 1)
        def _():
            v_start(b + 1)
        return carry

    jax.lax.fori_loop(0, B, batch, 0)


@jax.jit
def pallas_interleave_layers__sliding_block_cached__moe_arch_mod__decode_kernel(
    A_x: jax.Array,
    A_k_cache: jax.Array,
    A_v_cache: jax.Array,
    A_wq: jax.Array,
    A_wo: jax.Array,
    B_x: jax.Array,
    B_w_r: jax.Array,
    B_w_gate: jax.Array,
    B_w_up: jax.Array,
    B_w_down: jax.Array,
):
    del B_x
    kt = jnp.swapaxes(A_k_cache, 2, 3).reshape(B, NP, PD, SK)
    vt = jnp.swapaxes(A_v_cache, 2, 3).reshape(B, NP, PD, SK)
    out = pl.pallas_call(
        _kernel,
        out_shape=jax.ShapeDtypeStruct((B, D), BF),
        in_specs=[pl.BlockSpec(memory_space=pl.ANY)] * 9,
        out_specs=pl.BlockSpec(memory_space=pltpu.VMEM),
        scratch_shapes=[
            pltpu.VMEM((B, D), BF),
            pltpu.VMEM((NP, PD, W), BF),
            pltpu.VMEM((NP, PD, W), BF),
            pltpu.VMEM((D, H * DH), BF),
            pltpu.VMEM((NP, PD, D), BF),
            pltpu.VMEM((D // 128, 128), BF),
            pltpu.VMEM((D, F), BF),
            pltpu.VMEM((D, F), BF),
            pltpu.VMEM((F, D), BF),
            pltpu.VMEM((NP, PD // 2, W), U32),
            pltpu.VMEM((NP, PD, W), F32),
            pltpu.VMEM((D // 2, H * DH), U32),
            pltpu.VMEM((NP, WO_MXU // 2, D), U32),
            pltpu.VMEM((NP, WO_VPU, D), F32),
            pltpu.VMEM((D // 2, FA * 128), U32),
            pltpu.VMEM((D // 2, FA * 128), U32),
            pltpu.VMEM(((NF - KD) * 64, D), U32),
            pltpu.VMEM((D, (NF - FA) * 128), F32),
            pltpu.VMEM((D, (NF - FA) * 128), F32),
            pltpu.VMEM((KD * 128, D), F32),
            pltpu.VMEM((8, H * DH), F32),
            pltpu.VMEM((8, F), F32),
            pltpu.VMEM((8, F), F32),
            pltpu.VMEM((B, 8, D), F32),
            pltpu.VMEM((8, D), F32),
            pltpu.VMEM((NP, 16, W), F32),
            pltpu.VMEM((D, QV * PD), F32),
            pltpu.SemaphoreType.DMA((N_SEMS,)),
        ],
        compiler_params=pltpu.CompilerParams(vmem_limit_bytes=122 * 1024 * 1024,
                                             disable_semaphore_checks=True),
    )(A_x.reshape(B, D), kt, vt, A_wq, A_wo.reshape(NP, PD, D), B_w_r.reshape(D // 128, 128),
      B_w_gate, B_w_up, B_w_down)
    return out.reshape(B, 1, D)
```

```python
import math

import jax
import jax.numpy as jnp
import jax.experimental.pallas as pl
import jax.experimental.pallas.tpu as pltpu

B, D, H, DH, SK, F = 4, 640, 32, 192, 4096, 1536
W = 1024
NP = H // 2
PD = 2 * DH
NF = F // 128
EPS = 1e-5
BF = jnp.bfloat16
F32 = jnp.float32
U32 = jnp.uint32
EXP2_SCALE = (DH ** -0.5) * math.log2(math.e)

RG = 16
NG = PD // RG
LAST = (8, 8)
SEM_K = 7
SEM_V = 8
N_SEMS = SEM_V + NG - 1 + len(LAST)
WO_VPU = 256
WO_MXU = PD - WO_VPU
FA = 7
K0 = 1
KD = 6
QS = 2
QV = 4
DEP0 = 1
DEPN = 13


def _dot(a, b):
    return jnp.dot(a, b, preferred_element_type=F32)


def _bf(u):
    return pltpu.bitcast(u, BF)


def _fold(x):
    part = x[:, 0:128]
    for c in range(1, x.shape[1] // 128):
        part = part + x[:, 128 * c:128 * (c + 1)]
    return part


def _lanesum(x):
    return jnp.sum(_fold(x), axis=-1, keepdims=True)


def _rowsum(x):
    return jnp.broadcast_to(jnp.sum(x, axis=0, keepdims=True), x.shape)


def _stats(x, shift):
    d = x - shift
    both = jnp.concatenate([_fold(d), _fold(d * d)], axis=0)
    both = jnp.sum(both, axis=-1, keepdims=True) * (1.0 / D)
    md = both[0:8]
    var = jnp.maximum(both[8:16] - md * md, 0.0)
    return shift + md, jax.lax.rsqrt(var + EPS)


def _sigmoid(x):
    return 0.5 * jnp.tanh(0.5 * x) + 0.5


def _silu_mul(g, u):
    return g * _sigmoid(g) * u


def _recip(x):
    r = pl.reciprocal(x, approx=True)
    return r * (2.0 - x * r)


def _kernel(x_hbm, kt_hbm, vt_hbm, wq_hbm, wo_hbm, wr_hbm, wg_hbm, wu_hbm, wd_hbm,
            out_ref,
            xin, knat, vnat, wq_n, wo_n, wr, wg_n, wu_n, wd_n,
            ku, vf, wq, wo_u, wo_f, wg, wu, wd, wg_t, wu_t, wd_f,
            csq, csg, csu, xs, res, ps, wq_t, sems):
    win = pl.ds(SK - W, W)

    small = [pltpu.make_async_copy(x_hbm, xin, sems.at[0]),
             pltpu.make_async_copy(wr_hbm, wr, sems.at[1])]
    weights = [pltpu.make_async_copy(s, d, sems.at[2 + i]) for i, (s, d) in enumerate(
        [(wq_hbm, wq_n), (wo_hbm, wo_n), (wg_hbm, wg_n), (wu_hbm, wu_n), (wd_hbm, wd_n)])]

    def group_rows(j):
        return pl.ds(pl.multiple_of(j * RG, RG), RG)

    def k_start(b):
        def body(j, c):
            pltpu.make_async_copy(kt_hbm.at[b, :, group_rows(j), win],
                                  knat.at[:, group_rows(j)], sems.at[SEM_K]).start()
            return c
        jax.lax.fori_loop(0, NG, body, 0)

    def k_wait():
        pltpu.make_async_copy(knat, knat, sems.at[SEM_K]).wait()

    def v_group(b, j):
        return pltpu.make_async_copy(vt_hbm.at[b, :, group_rows(j), win],
                                     vnat.at[:, group_rows(j)], sems.at[SEM_V + j - 1])

    def v_piece(b, i):
        pairs = pl.ds(sum(LAST[:i]), LAST[i])
        return pltpu.make_async_copy(vt_hbm.at[b, pairs, pl.ds(0, RG), win],
                                     vnat.at[pairs, pl.ds(0, RG)],
                                     sems.at[SEM_V + NG - 1 + i])

    def v_start(b):
        def body(i, c):
            v_group(b, NG - 1 - i).start()
            return c
        jax.lax.fori_loop(0, NG - 1, body, 0)
        for i in range(len(LAST)):
            v_piece(b, i).start()

    for c in weights[:1] + small + weights[1:]:
        c.start()
    k_start(0)
    v_start(0)

    def pack_rows(src, dst, rows, cs):
        def body(i, c):
            r = pl.ds(pl.multiple_of(i * rows, 16), rows)
            r2 = pl.ds(pl.multiple_of(i * (rows // 2), 8), rows // 2)
            dst[r2, :] = pltpu.bitcast(src[r, cs], U32)
            return c
        jax.lax.fori_loop(0, src.shape[0] // rows, body, 0)

    def transpose_cols(src, dst, col0):
        def body(t, c):
            col = pl.ds(pl.multiple_of(col0 + t * 128, 128), 128)
            dst[pl.ds(pl.multiple_of(t * 128, 128), 128), :] = src[:, col].astype(F32).T
            return c
        jax.lax.fori_loop(0, dst.shape[0] // 128, body, 0)

    def col_sums(src, dst):
        def body(i, c):
            col = pl.ds(pl.multiple_of(i * 768, 128), 768)
            dst[:, col] = _dot(jnp.ones((8, D), BF), src[:, col])
            return c
        jax.lax.fori_loop(0, src.shape[1] // 768, body, 0)

    weights[0].wait()
    pack_rows(wq_n, wq, 16, slice(None))
    transpose_cols(wq_n, wq_t, QS * PD)
    col_sums(wq_n, csq)

    for c in small:
        c.wait()
    x_all = xin[...].astype(F32)
    for b in range(B):
        xs[b] = jnp.broadcast_to(x_all[b:b + 1, :], (8, D))
    res[...] = jnp.zeros((8, D), F32)

    weights[1].wait()

    def wo_body(g, c):
        wo_f[g] = wo_n[g, 0:WO_VPU, :].astype(F32)
        wo_u[g] = pltpu.bitcast(wo_n[g, WO_VPU:, :], U32)
        return c
    jax.lax.fori_loop(0, NP, wo_body, 0)

    for cp, src, dst_u, dst_t, cs in ((weights[2], wg_n, wg, wg_t, csg),
                                      (weights[3], wu_n, wu, wu_t, csu)):
        cp.wait()
        pack_rows(src, dst_u, 64, slice(0, FA * 128))
        transpose_cols(src, dst_t, FA * 128)
        col_sums(src, cs)

    weights[4].wait()

    def wd_body(t, c):
        r = pl.multiple_of(t * 128, 128)
        wd_f[pl.ds(r, 128), :] = wd_n[pl.ds(r + K0 * 128, 128), :].astype(F32)
        return c
    jax.lax.fori_loop(0, KD, wd_body, 0)
    wd[0:K0 * 64, :] = pltpu.bitcast(wd_n[0:K0 * 128, :], U32)
    wd[K0 * 64:, :] = pltpu.bitcast(wd_n[(K0 + KD) * 128:, :], U32)

    lane = jax.lax.broadcasted_iota(jnp.int32, (8, 128), 1)
    sub = jax.lax.broadcasted_iota(jnp.int32, (8, 128), 0)
    lane_pd = jax.lax.broadcasted_iota(jnp.int32, (8, PD), 1)
    sub_d = jax.lax.broadcasted_iota(jnp.int32, (8, D), 0)

    def cols(g):
        if isinstance(g, int):
            return slice(g * PD, (g + 1) * PD)
        return pl.ds(pl.multiple_of(g * PD, 128), PD)

    def scatter(o_cols):
        tiles = [jnp.zeros((8, 128), F32) for _ in range(len(o_cols) // 16)]
        for r, o_col in enumerate(o_cols):
            t, off = divmod(8 * r, 128)
            tiles[t] = jnp.where(lane == sub + off, o_col, tiles[t])
        return jnp.concatenate(tiles, axis=1)

    def matvec(x, w_ref):
        acc = None
        for r in range(w_ref.shape[0] // 8):
            t, off = divmod(8 * r, 128)
            col = jnp.sum(jnp.where(lane == sub + off, x[:, 128 * t:128 * (t + 1)], 0.0),
                          axis=-1, keepdims=True)
            p = col * w_ref[8 * r:8 * r + 8, :]
            acc = p if acc is None else acc + p
        return acc

    def matvec_t(x, wt_ref):
        return scatter([_lanesum(wt_ref[8 * r:8 * r + 8, :] * x)
                        for r in range(wt_ref.shape[0] // 8)])

    def split_heads(q):
        return jnp.concatenate([jnp.where(lane_pd < DH, q, 0.0),
                                jnp.where(lane_pd >= DH, q, 0.0)], axis=0).astype(BF)

    def q_proj(g, xb, m, rs):
        return split_heads((_dot(xb, _bf(wq[:, cols(g)])) - m * csq[:, cols(g)]) * rs)

    def ffn(x1, shift):
        x1b = x1.astype(BF)
        x1 = x1b.astype(F32)
        m1, rs1 = _stats(x1, shift)
        ag = matvec_t(x1, wg_t)
        au = matvec_t(x1, wu_t)
        hs = []
        for t in range(FA):
            cs = slice(128 * t, 128 * (t + 1))
            g = (_dot(x1b, _bf(wg[:, cs])) - m1 * csg[:, cs]) * rs1
            u = (_dot(x1b, _bf(wu[:, cs])) - m1 * csu[:, cs]) * rs1
            hs.append(_silu_mul(g, u))
        hv = _silu_mul((_rowsum(ag) - m1 * csg[:, FA * 128:]) * rs1,
                       (_rowsum(au) - m1 * csu[:, FA * 128:]) * rs1)
        yv = matvec(jnp.concatenate(hs[K0:K0 + KD], axis=1), wd_f)
        hm = jnp.concatenate(hs[:K0] + hs[K0 + KD:] + [hv], axis=1).astype(BF)
        ym = None
        for t in range(NF - KD):
            tm = _dot(hm[:, 128 * t:128 * (t + 1)], _bf(wd[64 * t:64 * (t + 1), :]))
            ym = tm if ym is None else ym + tm
        xn1 = (x1 - m1) * rs1
        wrf = wr[...].astype(F32)
        rp = xn1[:, 0:128] * wrf[0:1, :]
        for t in range(1, D // 128):
            rp = rp + xn1[:, 128 * t:128 * (t + 1)] * wrf[t:t + 1, :]
        gate = _sigmoid(jnp.sum(rp, axis=-1, keepdims=True))
        return x1 + xn1 + (ym + _rowsum(yv)) * gate, m1

    def attention2(x, shift):
        xb = x.astype(BF)
        m, rs = _stats(x, shift)
        rs = rs * EXP2_SCALE
        qs, runs, oms = {}, {}, []
        qv = (_rowsum(matvec_t(x, wq_t)) - m * csq[:, QS * PD:(QS + QV) * PD]) * rs
        for u in range(QV):
            qs[QS + u] = split_heads(qv[:, u * PD:(u + 1) * PD])
        acc = None
        for i in range(-2, NP):
            if i + 2 < NP and i + 2 not in qs:
                qs[i + 2] = q_proj(i + 2, xb, m, rs)
            g = i + 1
            if 0 <= g < NP:
                run = None
                for c in range(W // 128):
                    cs = slice(c * 128, (c + 1) * 128)
                    d = [_dot(qs[g][:, 128 * k:128 * (k + 1)],
                              _bf(ku[g, 64 * k:64 * (k + 1), cs])) for k in range(3)]
                    sc = jnp.concatenate([d[0][0:8] + d[1][0:8], d[1][8:16] + d[2][8:16]],
                                         axis=0)
                    ps[g, :, cs] = sc
                    run = sc if run is None else jnp.maximum(run, sc)
                runs[g] = (run, jnp.max(run, axis=-1, keepdims=True))
            if i >= 0:
                rest = []
                for hh in range(2):
                    mx = runs[i][1][8 * hh:8 * hh + 8]
                    if DEP0 <= i < DEPN:
                        mx = jnp.maximum(mx, jnp.minimum(runs[i + 1][0][0:8], mx))
                        mx = jnp.concatenate([mx] * (W // 128), axis=1)
                    ph = jnp.exp2(ps[i, 8 * hh:8 * hh + 8, :] - mx)
                    inv = _recip(_lanesum(ph))
                    acc_h = None
                    for r in range(hh * (DH // 8), (hh + 1) * (DH // 8)):
                        o_col = _lanesum(vf[i, 8 * r:8 * r + 8, :] * ph)
                        if 8 * r < WO_VPU:
                            t = o_col * wo_f[i, 8 * r:8 * r + 8, :]
                            acc_h = t if acc_h is None else acc_h + t
                        else:
                            rest.append(o_col)
                    acc = acc_h * inv if acc is None else acc + acc_h * inv
                oms.append((scatter(rest) * inv).astype(BF))
        acc2 = None
        for i in range(NP):
            t = _dot(oms[i], _bf(wo_u[i]))
            acc2 = t if acc2 is None else acc2 + t
        return acc + acc2, m

    def batch(b, carry):
        x = xs[b]

        k_wait()

        def body_k(i, c):
            g = i // 4
            r = pl.multiple_of((i % 4) * 96, 16)
            ku[g, pl.ds(pl.multiple_of((i % 4) * 48, 8), 48), :] = pltpu.bitcast(
                knat[g, pl.ds(r, 96), :], U32)
            return c
        jax.lax.fori_loop(0, NP * 4, body_k, 0)

        @pl.when(b < B - 1)
        def _():
            k_start(b + 1)

        xb = x.astype(BF)
        m, rs = _stats(x, jnp.mean(x, axis=-1, keepdims=True))
        rs = rs * EXP2_SCALE

        def body_a(i, c):
            qs = [q_proj(4 * i + u, xb, m, rs) for u in range(4)]
            for u in range(4):
                s = _dot(qs[u], _bf(ku[4 * i + u]))
                p = jnp.exp2(s - jnp.max(s, axis=-1, keepdims=True))
                ps[4 * i + u] = p * _recip(jnp.sum(p, axis=-1, keepdims=True))
            return c
        jax.lax.fori_loop(0, NP // 4, body_a, 0)

        def pv1(pairs, row0, hrow):
            out = []
            for g in pairs:
                ph = ps[g, pl.ds(hrow, 8), :]
                for t in range(RG // 8):
                    rows = pl.ds(row0 + 8 * t, 8)
                    v = vnat[g, rows, :].astype(F32)
                    vf[g, rows, :] = v
                    out.append(_lanesum(v * ph))
            return out

        def o_proj(j, o):
            return _dot(o, wo_n[:, group_rows(j), :].reshape(NP * RG, D))

        def body_b(i, c):
            acc, o_prev = c
            j = NG - 1 - i
            v_group(b, j).wait()
            acc = acc + o_proj(jnp.minimum(j + 1, NG - 1), o_prev)
            hrow = pl.multiple_of(jnp.where(j * RG >= DH, 8, 0), 8)
            o_cols = pv1(range(NP), pl.multiple_of(j * RG, RG), hrow)
            return acc, scatter(o_cols).astype(BF)
        acc, o_prev = jax.lax.fori_loop(
            0, NG - 1, body_b, (jnp.zeros((8, D), F32), jnp.zeros((8, NP * RG), BF)))

        for i in range(len(LAST)):
            v_piece(b, i).wait()
            if i == 0:
                acc = acc + o_proj(1, o_prev)
            g0 = sum(LAST[:i])
            for k, o_col in enumerate(pv1(range(g0, g0 + LAST[i]), 0, 0)):
                g, t = divmod(k, RG // 8)
                acc = acc + o_col * wo_f[g0 + g, 8 * t:8 * t + 8, :]

        x, m = ffn(x + _rowsum(acc), m)
        x = x.astype(BF).astype(F32)
        acc, m = attention2(x, m)
        x, _ = ffn(x + _rowsum(acc), m)
        r = jnp.where(sub_d == b, x, res[...])
        res[...] = r
        out_ref[...] = r[0:B, :].astype(BF)

        @pl.when(b < B - 1)
        def _():
            v_start(b + 1)
        return carry

    jax.lax.fori_loop(0, B, batch, 0)


@jax.jit
def pallas_interleave_layers__sliding_block_cached__moe_arch_mod__decode_kernel(
    A_x: jax.Array,
    A_k_cache: jax.Array,
    A_v_cache: jax.Array,
    A_wq: jax.Array,
    A_wo: jax.Array,
    B_x: jax.Array,
    B_w_r: jax.Array,
    B_w_gate: jax.Array,
    B_w_up: jax.Array,
    B_w_down: jax.Array,
):
    del B_x
    kt = jnp.swapaxes(A_k_cache, 2, 3).reshape(B, NP, PD, SK)
    vt = jnp.swapaxes(A_v_cache, 2, 3).reshape(B, NP, PD, SK)
    out = pl.pallas_call(
        _kernel,
        out_shape=jax.ShapeDtypeStruct((B, D), BF),
        in_specs=[pl.BlockSpec(memory_space=pl.ANY)] * 9,
        out_specs=pl.BlockSpec(memory_space=pltpu.VMEM),
        scratch_shapes=[
            pltpu.VMEM((B, D), BF),
            pltpu.VMEM((NP, PD, W), BF),
            pltpu.VMEM((NP, PD, W), BF),
            pltpu.VMEM((D, H * DH), BF),
            pltpu.VMEM((NP, PD, D), BF),
            pltpu.VMEM((D // 128, 128), BF),
            pltpu.VMEM((D, F), BF),
            pltpu.VMEM((D, F), BF),
            pltpu.VMEM((F, D), BF),
            pltpu.VMEM((NP, PD // 2, W), U32),
            pltpu.VMEM((NP, PD, W), F32),
            pltpu.VMEM((D // 2, H * DH), U32),
            pltpu.VMEM((NP, WO_MXU // 2, D), U32),
            pltpu.VMEM((NP, WO_VPU, D), F32),
            pltpu.VMEM((D // 2, FA * 128), U32),
            pltpu.VMEM((D // 2, FA * 128), U32),
            pltpu.VMEM(((NF - KD) * 64, D), U32),
            pltpu.VMEM(((NF - FA) * 128, D), F32),
            pltpu.VMEM(((NF - FA) * 128, D), F32),
            pltpu.VMEM((KD * 128, D), F32),
            pltpu.VMEM((8, H * DH), F32),
            pltpu.VMEM((8, F), F32),
            pltpu.VMEM((8, F), F32),
            pltpu.VMEM((B, 8, D), F32),
            pltpu.VMEM((8, D), F32),
            pltpu.VMEM((NP, 16, W), F32),
            pltpu.VMEM((QV * PD, D), F32),
            pltpu.SemaphoreType.DMA((N_SEMS,)),
        ],
        compiler_params=pltpu.CompilerParams(vmem_limit_bytes=122 * 1024 * 1024,
                                             disable_semaphore_checks=True),
    )(A_x.reshape(B, D), kt, vt, A_wq, A_wo.reshape(NP, PD, D), B_w_r.reshape(D // 128, 128),
      B_w_gate, B_w_up, B_w_down)
    return out.reshape(B, 1, D)
```
